```python
import os as _os
_os.environ.setdefault("JAX_PLATFORMS", "cpu")
import jax
import jax.numpy as jnp

def _softmax(x, axis=-1):
    return jax.nn.softmax(x, axis=axis)
def _gelu(x):
    return jax.nn.gelu(x, approximate=True)
def _silu(x):
    return jax.nn.silu(x)
def _sigmoid(x):
    return jax.nn.sigmoid(x)
def _layernorm(x, axis=-1, eps=1e-5):
    m = jnp.mean(x, axis=axis, keepdims=True)
    v = jnp.var(x, axis=axis, keepdims=True)
    return (x - m) / jnp.sqrt(v + eps)
def _scatter_add(tgt, idx, src, axis=0):
    return tgt.at[idx].add(src)
def _segment_sum(src, seg, n):
    return jax.ops.segment_sum(src, seg, n)
class _Rng:
    def __init__(self, key):
        self._k = key
    def _next(self):
        self._k, sub = jax.random.split(self._k)
        return sub
    def normal(self, shape):
        return jax.random.normal(self._next(), shape, dtype=jnp.bfloat16)
    def randint(self, lo, hi, shape):
        return jax.random.randint(self._next(), shape, lo, hi, dtype=jnp.int32)
    def uniform(self, shape, lo=0.0, hi=1.0):
        return jax.random.uniform(self._next(), shape, jnp.bfloat16, lo, hi)
    def permutation(self, n):
        return jax.random.permutation(self._next(), n)


kernel_name = 'gated_mix__ssm_conv_h3__linear_kernel_hedgehog__prompt'

def setup_inputs():
    _rng = _Rng(jax.random.key(int.from_bytes(__import__("os").urandom(4), "little")))
    _w = (lambda a: (lambda t: t.astype(jnp.bfloat16) if jnp.issubdtype(t.dtype, jnp.floating) else t)(jnp.asarray(a)))
    def _A_setup():
        B, S, D = 1, 2048, 576
        ks = 4
        return {
            "q": _w((lambda *s: _rng.normal(s) * 0.05)(B, S, D)),
            "k": _w((lambda *s: _rng.normal(s) * 0.4)(B, S, D)),
            "v": _w((lambda *s: _rng.normal(s) * 0.4)(B, S, D)),
            "shift_k": _w((lambda *s: _rng.normal(s) * 0.4)(D, ks) * 0.5),
            "ssm_k": _w((lambda *s: _rng.normal(s) * 0.4)(D, S) * (1.0 / S ** 0.5)),
            "ssm_D": _w((lambda *s: _rng.normal(s) * 0.4)(D)),
        }
    _A_in = _A_setup()

    def _B_setup():
        B, S, D, H = 1, 2048, 576, 32
        Dh = D // H
        return {
            "x": _w((lambda *s: _rng.normal(s) * 0.05)(B, S, D)),
            "wqkv": _w((lambda *s: _rng.normal(s) * 0.8)(D, 3 * D)),
            "w_phi": _w((lambda *s: _rng.normal(s) * 0.8)(H, Dh, Dh) * (Dh ** -0.5)),
            "wo": _w((lambda *s: _rng.normal(s) * 0.05)(D, D)),
        }
    _B_in = _B_setup()

    return {
        "A_q": _A_in["q"],
        "A_k": _A_in["k"],
        "A_v": _A_in["v"],
        "A_shift_k": _A_in["shift_k"],
        "A_ssm_k": _A_in["ssm_k"],
        "A_ssm_D": _A_in["ssm_D"],
        "B_x": _B_in["x"],
        "B_wqkv": _B_in["wqkv"],
        "B_w_phi": _B_in["w_phi"],
        "B_wo": _B_in["wo"],
        "gate_w": _w((lambda *s: _rng.normal(s) * 0.05)(576) * 16.0),
    }

def reference(A_q, A_k, A_v, A_shift_k, A_ssm_k, A_ssm_D, B_x, B_wqkv, B_w_phi, B_wo, gate_w):
    def _A_ref(q, k, v, shift_k, ssm_k, ssm_D):
        B, S, D = q.shape
        ks = shift_k.shape[-1]
        k_pad = jnp.pad(k, ((0, 0), (ks - 1, 0), (0, 0)))
        k_shift = jnp.zeros_like(k)
        for t in range(ks):
            k_shift = k_shift + k_pad[:, t:t + S, :] * shift_k[:, ks - 1 - t][None, None, :]
        kv = k_shift * v
        L = 2 * S
        kv_pad = jnp.pad(kv, ((0, 0), (0, S), (0, 0)))
        kf_pad = jnp.pad(ssm_k, ((0, 0), (0, S)))
        kv_f = (lambda x, axes=(-2,-1): jnp.fft.rfft2(x.astype(jnp.float32), axes=axes))(kv_pad[:, None, :, :], axes=(1, 2))
        kf_f = (lambda x, axes=(-2,-1): jnp.fft.rfft2(x.astype(jnp.float32), axes=axes))(kf_pad[:, None, :], axes=(1, 2))
        kf_f = (lambda x, *d: x.transpose(*d))(kf_f, 1, 2, 0)
        y_f = kv_f * kf_f[None, :, :, :]
        y = (lambda x, s, axes=(-2,-1): jnp.fft.irfft2(x, s=s, axes=axes).astype(jnp.bfloat16))(y_f, (1, L), axes=(1, 2))[:, 0, :S, :]
        y = y + kv * ssm_D[None, None, :]
        return q * y

    def _B_ref(x, wqkv, w_phi, wo):
        B, S, D = x.shape
        H = 32; Dh = D // H
        qkv = (lambda x, *d: x.transpose(*d))((x @ wqkv).reshape(B, S, 3, H, Dh), 2, 0, 3, 1, 4)
        q, k, v = qkv[0], qkv[1], qkv[2]
        pq = jnp.einsum("bhsd,hdf->bhsf", q, w_phi)
        pk = jnp.einsum("bhsd,hdf->bhsf", k, w_phi)
        phi_q = jnp.concatenate([_softmax(pq, axis=-1), _softmax(-pq, axis=-1)], axis=-1)
        phi_k = jnp.concatenate([_softmax(pk, axis=-1), _softmax(-pk, axis=-1)], axis=-1)
        kv = jnp.einsum("bhsf,bhsd->bhfd", phi_k, v)
        z  = jnp.einsum("bhsf->bhf", phi_k)
        num = jnp.einsum("bhqf,bhfd->bhqd", phi_q, kv)
        den = jnp.einsum("bhqf,bhf->bhq", phi_q, z)[..., None] + 1e-6
        o = num / den
        return (lambda x, *d: x.transpose(*d))(o, 0, 2, 1, 3).reshape(B, S, D) @ wo

    x = A_q
    g = _sigmoid((x * gate_w).sum(-1, keepdims=True))
    a = _A_ref(x, A_k, A_v, A_shift_k, A_ssm_k, A_ssm_D)
    b = _B_ref(x, B_wqkv, B_w_phi, B_wo)
    return g * a + (1 - g) * b
```

```python
import numpy as np
import jax
import jax.numpy as jnp
from jax import lax
from jax.experimental import pallas as pl
from jax.experimental.pallas import tpu as pltpu

S = 2048
D = 576
DH = 18
BL = 128
NB = S // BL
RC = 64
NC = D // RC
TS = 256
NS = S // TS
GR = 4 * DH
NG = D // GR
NT = 2 * D // 128
LOG2E = 1.4426950408889634

F32 = jnp.float32
BF16 = jnp.bfloat16
_NT_DIMS = (((1,), (1,)), ((), ()))


def _dft_consts():
    k = np.arange(BL, dtype=np.float64)
    n = np.arange(BL, dtype=np.float64)
    ang = np.outer(n, np.pi * (4.0 * k + 1.0) / (2.0 * BL))
    fwd = np.concatenate([np.cos(ang), np.sin(ang)], axis=1)
    inv = np.concatenate([np.cos(ang).T, np.sin(ang).T], axis=0) / BL
    return fwd.astype(np.float32), inv.astype(np.float32)


def _vwin(t):
    lo = max(GR * (t - 1), 0)
    hi = min(GR * (t + 1), D)
    return lo, hi, (lo // 16) * 16, -(-hi // 16) * 16


def _dot(a, b):
    return jnp.dot(a, b, preferred_element_type=F32)


def _dot_nt(a, b):
    return lax.dot_general(a, b, _NT_DIMS, preferred_element_type=F32)


def _conv16(xs, hs, init, sub):
    out = []
    for m in range(NB):
        acc = None if init is None else init[m]
        for i in range(m + 1):
            p = xs[i] * hs[m - i]
            if acc is None:
                acc = p
            elif sub:
                acc = acc - p
            else:
                acc = acc + p
        out.append(acc)
    return out


def _group_exp(p):
    w = p.shape[1]
    p3 = p.reshape(9, 8, w)
    mx = jnp.max(p3, axis=0)
    mx = jnp.maximum(mx, pltpu.roll(mx, 4, 0))
    mn = jnp.min(p3, axis=0)
    mn = jnp.minimum(mn, pltpu.roll(mn, 4, 0))
    ep = jnp.exp2(p3 - mx[None])
    en = jnp.exp2(mn[None] - p3)
    sp = jnp.sum(ep, axis=0)
    sp = sp + pltpu.roll(sp, 4, 0)
    sn = jnp.sum(en, axis=0)
    sn = sn + pltpu.roll(sn, 4, 0)
    return ep, en, sp, sn


def _kernel(x_hbm, k_hbm, v_hbm, sk_hbm, h_hbm, d_hbm, wqkv_hbm, wp_hbm, wo_hbm, gate_hbm,
            f_hbm, g_hbm, out_hbm,
            xbuf, kbuf, vbuf, hbuf, wqkv, wo, skb, db, gb, wpb, fm, gm,
            wp2, wt, wot, wb, uh, zs, ybuf, phik, kvacc, zacc, lhs, obuf,
            sem_small, sem_w, sem_x, sem_k, sem_v, sem_h, sem_o):
    small = [
        pltpu.make_async_copy(wp_hbm, wpb, sem_small.at[0]),
        pltpu.make_async_copy(sk_hbm, skb, sem_small.at[1]),
        pltpu.make_async_copy(d_hbm, db, sem_small.at[2]),
        pltpu.make_async_copy(gate_hbm, gb, sem_small.at[3]),
        pltpu.make_async_copy(f_hbm, fm, sem_small.at[4]),
        pltpu.make_async_copy(g_hbm, gm, sem_small.at[5]),
    ]
    for c in small:
        c.start()

    def cp_k(c):
        return pltpu.make_async_copy(k_hbm.at[0, pl.ds(c * RC, RC), :], kbuf.at[c], sem_k.at[c])

    def cp_v(c):
        return pltpu.make_async_copy(v_hbm.at[0, pl.ds(c * RC, RC), :], vbuf.at[c], sem_v.at[c])

    def cp_h(c):
        return pltpu.make_async_copy(h_hbm.at[pl.ds(c * RC, RC), :], hbuf.at[c], sem_h.at[c])

    def cp_x(i):
        return pltpu.make_async_copy(x_hbm.at[0, :, pl.ds(i * TS, TS)], xbuf.at[i], sem_x.at[i])

    def cp_o(i):
        return pltpu.make_async_copy(obuf.at[i], out_hbm.at[0, :, pl.ds(i * TS, TS)], sem_o.at[i])

    cp_w = pltpu.make_async_copy(wqkv_hbm, wqkv, sem_w.at[0])
    cp_wo = pltpu.make_async_copy(wo_hbm, wo, sem_w.at[1])

    cp_k(0).start(); cp_v(0).start(); cp_h(0).start()
    cp_w.start()
    for i in range(NS):
        cp_x(i).start()
        cp_k(i + 1).start(); cp_v(i + 1).start(); cp_h(i + 1).start()
    cp_wo.start()

    for c in small:
        c.wait()

    sk = skb[...].astype(F32)
    for j in range(4):
        wb[j] = jnp.broadcast_to(sk[j:j + 1, :], (128, D)).T
    wb[4] = jnp.broadcast_to(db[...].astype(F32).reshape(1, D), (128, D)).T
    wb[5] = jnp.broadcast_to(gb[...].astype(F32).reshape(1, D), (128, D)).T

    lane16 = lax.broadcasted_iota(jnp.int32, (16, 128), 1)

    def conv_chunk(c):
        r0 = c * RC if isinstance(c, int) else pl.multiple_of(c * RC, RC)
        cp_k(c).wait(); cp_v(c).wait(); cp_h(c).wait()
        ublk = [[None] * (RC // 16) for _ in range(NB)]
        for rs in range(RC // 16):
            w0, w1, w2, w3 = [wb[j, pl.ds(r0 + rs * 16, 16), :] for j in range(4)]
            r1p = jnp.zeros((16, 128), F32)
            r2p = jnp.zeros((16, 128), F32)
            for i in range(NB):
                kt = kbuf[c, rs * 16:(rs + 1) * 16, i * BL:(i + 1) * BL].astype(F32)
                vt = vbuf[c, rs * 16:(rs + 1) * 16, i * BL:(i + 1) * BL].astype(F32)
                r1 = pltpu.roll(kt, 1, 1)
                k1 = jnp.where(lane16 >= 1, r1, r1p)
                t = w2 * kt + w3 * k1
                r2 = pltpu.roll(t, 2, 1)
                t2 = jnp.where(lane16 >= 2, r2, r2p)
                ks = w0 * kt + w1 * k1 + t2
                ublk[i][rs] = (ks * vt).astype(BF16)
                r1p, r2p = r1, r2
        ust = jnp.concatenate([ublk[i][rs] for i in range(NB) for rs in range(RC // 16)], axis=0)
        hst = jnp.concatenate([hbuf[c, :, i * BL:(i + 1) * BL] for i in range(NB)], axis=0)
        fmat = fm[...]
        uh[0:NB * RC, :] = _dot(ust, fmat)
        uh[NB * RC:2 * NB * RC, :] = _dot(hst, fmat)
        for p in range(RC // 8):
            def ld(base, i, half):
                return uh[base + i * RC + p * 8: base + i * RC + p * 8 + 8, half * 128:(half + 1) * 128]
            dcol = wb[4, pl.ds(r0 + p * 8, 8), :]
            hb = NB * RC
            cs = [ld(hb, j, 0) for j in range(NB)]
            cs[0] = cs[0] + dcol
            ss = [ld(0, i, 0) + ld(0, i, 1) for i in range(NB)]
            k1 = _conv16(ss, cs, None, False)
            qs = [cs[j] + ld(hb, j, 1) for j in range(NB)]
            bs = [ld(0, i, 1) for i in range(NB)]
            re = _conv16(bs, qs, k1, True)
            ps = [ld(hb, j, 1) - cs[j] for j in range(NB)]
            as_ = [ld(0, i, 0) for i in range(NB)]
            im = _conv16(as_, ps, k1, False)
            for m in range(NB):
                zr = re[m] if m == 0 else re[m] + im[m - 1]
                zi = im[m] if m == 0 else im[m] - re[m - 1]
                zs[m * RC + p * 8: m * RC + p * 8 + 8, 0:128] = zr
                zs[m * RC + p * 8: m * RC + p * 8 + 8, 128:256] = zi
        y = _dot(zs[...].astype(BF16), gm[...])
        for m in range(NB):
            ybuf[m, pl.ds(r0, RC), :] = y[m * RC:(m + 1) * RC]

    conv_chunk(0)

    eye = (lax.broadcasted_iota(jnp.int32, (32, 32), 0)
           == lax.broadcasted_iota(jnp.int32, (32, 32), 1)).astype(BF16)
    for e in range(DH):
        t = _dot_nt(eye, wpb[e])
        wp2[pl.ds(e, 32, stride=DH), :] = t
        wp2[pl.ds(D + e, 32, stride=DH), :] = t
    rep = ((lax.broadcasted_iota(jnp.int32, (GR, DH), 0) >> 2)
           == lax.broadcasted_iota(jnp.int32, (GR, DH), 1)).astype(BF16)
    a2 = _dot_nt(rep, wp2[...].astype(BF16))
    row4 = lax.broadcasted_iota(jnp.int32, (GR, 128), 0) & 3
    lane72 = lax.broadcasted_iota(jnp.int32, (GR, 128), 1)
    cp_w.wait()
    parts = {}
    for t in range(NT):
        g_lo = (128 * t) // GR
        g_hi = (128 * t + 127) // GR
        at = a2[:, 128 * t:128 * (t + 1)]
        blocks = []
        for gg in range(g_lo, g_hi + 1):
            lo = (4 * gg + row4) * DH - 128 * t
            blocks.append(jnp.where((lane72 >= lo) & (lane72 < lo + DH), at, 0.0))
        lt = jnp.concatenate(blocks, axis=0).astype(BF16)
        res = _dot_nt(lt, wqkv[:, 128 * t:128 * (t + 1)])
        for n, gg in enumerate(range(g_lo, g_hi + 1)):
            piece = res[GR * n:GR * (n + 1)]
            parts[gg] = piece if gg not in parts else parts[gg] + piece
    for gp in range(NG):
        pair = jnp.concatenate([parts[2 * gp], parts[2 * gp + 1]], axis=0) * LOG2E
        wt[2 * GR * gp:2 * GR * (gp + 1), :] = pair.astype(BF16)
    wt[2 * D:3 * D, :] = wqkv[:, 2 * D:3 * D].T

    kvacc[...] = jnp.zeros(kvacc.shape, F32)
    zacc[...] = jnp.zeros(zacc.shape, F32)

    def loop1(i, carry):
        cp_x(i).wait()
        xt = xbuf[i]
        for gp in range(NG // 2):
            pk = _dot(wt[D + 2 * GR * gp: D + 2 * GR * (gp + 1), :], xt)
            for gi in range(2):
                g = 2 * gp + gi
                ep, en, sp, sn = _group_exp(pk[GR * gi:GR * (gi + 1)])
                pp = (ep * (1.0 / sp)[None]).reshape(GR, TS)
                pn = (en * (1.0 / sn)[None]).reshape(GR, TS)
                ph = jnp.concatenate([pp, pn], axis=0)
                phik[2 * GR * g:2 * GR * (g + 1), :] = ph.astype(BF16)
                zpart = ph[:, 0:128]
                for q in range(1, TS // 128):
                    zpart = zpart + ph[:, 128 * q:128 * (q + 1)]
                zacc[2 * GR * g:2 * GR * (g + 1), :] += zpart
        vt = _dot(wt[2 * D:3 * D, :], xt).astype(BF16)
        for t in range(NT):
            _, _, lo, hi = _vwin(t)
            kvacc[t, 0:hi - lo, :] += _dot_nt(vt[lo:hi], phik[128 * t:128 * (t + 1), :])
        conv_chunk(i + 1)
        return carry

    lax.fori_loop(0, NS, loop1, 0)

    zacc[...] = jnp.broadcast_to(jnp.sum(zacc[...], axis=1, keepdims=True), zacc.shape)
    for t in range(NT):
        lo, hi, alo, _ = _vwin(t)
        n = hi - lo
        kvt = kvacc[t, lo - alo:lo - alo + n, :]
        lane = lax.broadcasted_iota(jnp.int32, (n, 128), 1)
        vrow = lax.broadcasted_iota(jnp.int32, (n, 128), 0) + lo
        hd = jnp.where(lane < 16 * t, 4 * (t - 1), 4 * t) + (lane & 3)
        keep = (vrow >= hd * DH) & (vrow < hd * DH + DH)
        lhs[t, 0:n, :] = jnp.where(keep, kvt, 0.0).astype(BF16)
    cp_wo.wait()
    wot[...] = wo[...].T

    def loop2(i, carry):
        xt = xbuf[i]
        for gp in range(NG // 2):
            pq = _dot(wt[2 * GR * gp:2 * GR * (gp + 1), :], xt)
            for gi in range(2):
                g = 2 * gp + gi
                ep, en, sp, sn = _group_exp(pq[GR * gi:GR * (gi + 1)])
                zp = zacc[2 * GR * g:2 * GR * g + GR, :].reshape(9, 8, 128)
                zn = zacc[2 * GR * g + GR:2 * GR * (g + 1), :].reshape(9, 8, 128)
                zp = jnp.concatenate([zp] * (TS // 128), axis=2)
                zn = jnp.concatenate([zn] * (TS // 128), axis=2)
                tp = jnp.sum(ep * zp, axis=0)
                tp = tp + pltpu.roll(tp, 4, 0)
                tn = jnp.sum(en * zn, axis=0)
                tn = tn + pltpu.roll(tn, 4, 0)
                rp = 1.0 / sp
                rn = 1.0 / sn
                rden = 1.0 / (tp * rp + tn * rn + 1e-6)
                pp = (ep * (rp * rden)[None]).reshape(GR, TS)
                pn = (en * (rn * rden)[None]).reshape(GR, TS)
                phik[2 * GR * g:2 * GR * (g + 1), :] = jnp.concatenate([pp, pn], axis=0).astype(BF16)
        res = []
        for t in range(NT):
            lo, hi, _, _ = _vwin(t)
            res.append(_dot(lhs[t, 0:hi - lo, :], phik[128 * t:128 * (t + 1), :]))
        og = []
        for g in range(NG):
            a = res[g] if g == 0 else res[g][GR:2 * GR]
            og.append(a + res[g + 1][0:GR])
        ot = jnp.concatenate(og, axis=0).astype(BF16)
        bt = _dot(wot[...], ot)
        xf = xt.astype(F32)
        gw = wb[5]
        gw = jnp.concatenate([gw] * (TS // 128), axis=1)
        gl = jnp.sum((xf * gw).reshape(D // 8, 8, TS), axis=0)
        gl = jnp.sum(gl, axis=0, keepdims=True)
        gate = 1.0 / (1.0 + jnp.exp(-gl))
        y = jnp.concatenate([ybuf[(TS // 128) * i + q] for q in range(TS // 128)], axis=1)
        o = bt + gate * (xf * y - bt)
        obuf[i] = o.astype(BF16)
        cp_o(i).start()
        return carry

    lax.fori_loop(0, NS, loop2, 0)
    for i in range(NS):
        cp_o(i).wait()


@jax.jit
def pallas_gated_mix__ssm_conv_h3__linear_kernel_hedgehog__prompt_kernel(A_q, A_k, A_v, A_shift_k, A_ssm_k, A_ssm_D, B_x, B_wqkv, B_w_phi, B_wo, gate_w):
    del B_x
    fwd, inv = _dft_consts()
    xT = jnp.transpose(A_q, (0, 2, 1))
    kT = jnp.transpose(A_k, (0, 2, 1))
    vT = jnp.transpose(A_v, (0, 2, 1))
    skT = jnp.transpose(A_shift_k, (1, 0))
    wp = jnp.transpose(B_w_phi, (1, 2, 0))
    hbm = pl.BlockSpec(memory_space=pltpu.HBM)
    scratch = [
        pltpu.VMEM((NS, D, TS), BF16),
        pltpu.VMEM((NC, RC, S), BF16),
        pltpu.VMEM((NC, RC, S), BF16),
        pltpu.VMEM((NC, RC, S), BF16),
        pltpu.VMEM((D, 3 * D), BF16),
        pltpu.VMEM((D, D), BF16),
        pltpu.VMEM((4, D), BF16),
        pltpu.VMEM((D,), BF16),
        pltpu.VMEM((D,), BF16),
        pltpu.VMEM((DH, DH, 32), BF16),
        pltpu.VMEM((BL, 2 * BL), BF16),
        pltpu.VMEM((2 * BL, BL), BF16),
        pltpu.VMEM((2 * D, DH), F32),
        pltpu.VMEM((3 * D, D), BF16),
        pltpu.VMEM((D, D), BF16),
        pltpu.VMEM((6, D, 128), F32),
        pltpu.VMEM((2 * NB * RC, 2 * BL), F32),
        pltpu.VMEM((NB * RC, 2 * BL), F32),
        pltpu.VMEM((NB, D, BL), F32),
        pltpu.VMEM((2 * D, TS), BF16),
        pltpu.VMEM((NT, 160, 128), F32),
        pltpu.VMEM((2 * D, 128), F32),
        pltpu.VMEM((NT, 2 * GR, 128), BF16),
        pltpu.VMEM((NS, D, TS), BF16),
        pltpu.SemaphoreType.DMA((6,)),
        pltpu.SemaphoreType.DMA((2,)),
        pltpu.SemaphoreType.DMA((NS,)),
        pltpu.SemaphoreType.DMA((NC,)),
        pltpu.SemaphoreType.DMA((NC,)),
        pltpu.SemaphoreType.DMA((NC,)),
        pltpu.SemaphoreType.DMA((NS,)),
    ]
    outT = pl.pallas_call(
        _kernel,
        out_shape=jax.ShapeDtypeStruct((1, D, S), BF16),
        in_specs=[hbm] * 12,
        out_specs=hbm,
        scratch_shapes=scratch,
        compiler_params=pltpu.CompilerParams(vmem_limit_bytes=100 * 1024 * 1024),
    )(xT, kT, vT, skT, A_ssm_k, A_ssm_D, B_wqkv, wp, B_wo, gate_w,
      jnp.asarray(fwd, BF16), jnp.asarray(inv, BF16))
    return jnp.transpose(outT, (0, 2, 1))
```

```python
import numpy as np
import jax
import jax.numpy as jnp
from jax import lax
from jax.experimental import pallas as pl
from jax.experimental.pallas import tpu as pltpu

S = 2048
D = 576
DH = 18
BL = 128
NB = S // BL
HB = NB // 2
RC = 64
NC = D // RC
TS = 256
NS = S // TS
NQ = TS // 128
GR = 4 * DH
NG = D // GR
NT = 2 * D // 128
PR = 48
NP = D // PR
P1 = 64
JR = 64
DP = 1024
GP = 72
FQ = 3
OR = 136
QK = 8 * OR
FR = OR + 8
NPAIR = 16
KW = 48
KF = 80
KVA = 6
BM = 4
XN = 4
OSPLIT = (8, 11, 12)
LOG2E = 1.4426950408889634

ORDER = {
    's1': (
        'q q f q f q q q '),
    's2': (
        'q f f f q q q q q f q '),
    's3': (
        'h h q u h h u h q h u u q h h u h u q u u h h q u u h q h u h u h u q u q h u u '),
    's4': (
        'qB qB qBB qBB qBB qBB qB qB qBB qB qB qB qB '),
    's5': (
        'vG hB h vB v u hG vB hB u v hG u v hB u vB hB u v hB u vB hG u vB hG u vB h u vB hG u v h uB v '
        'hB uG v hB uG v hB u v uB v uB '),
    'ma': (
        'm0 m m m130 m m2 m0 m1 m0 m m32 m m0 m13 m m0 m1 m m0 m0 m3 m m10 m20 m m3 m0 m m10 m m m1 m '
        'm302 m m0 m m1 m m3 m30 m2 m m1 m m0 m m '),
    'x': (
        'm2 m m m1 m m1 m m m0 m0 m m m m m2 m m1 m1 m m0 m m m m2 m m1 m m m1 m m0 m m m2 m m m1 m0 m m '
        'm1 m m2 m m m m m0 m2 m m m1 m m0 m m1 m m m2 m m1 m m m m0 m m2 m m1 m m m1 m m0 m m m2 m m m1 '
        'm m0 m m2 m m m1 m m1 m m0 m m m2 m m m1 m m m2 m m0 m m1 m m m1 m m0 m m m1 m m2 m m m m m2 m0 '
        'm1 m m m m1 m0 m m m2 m m m m1 m2 m m m0 m m m m1 m m m '),
    'loop': (
        'vS hB qB v qB uS qS hB qS u qB hS v uBS v qB qS h qBS vS u qB qB hS q uBS q h vB vBS u q hSS q '
        'uB vB vB uBS q h qS qB vS u qBS h qB vB u qBS q vBSS h q u hBS q vB qB u qS hB vS uS q qBS h vB '
        'uB qBS h v qB qS uS vS h qB vB qS uBS h q qB '),
}

F32 = jnp.float32
BF16 = jnp.bfloat16
U32 = jnp.uint32
_NT_DIMS = (((1,), (1,)), ((), ()))


def _dft_consts():
    k = np.arange(BL, dtype=np.float64)
    n = np.arange(BL, dtype=np.float64)
    ang = np.outer(n, np.pi * (4.0 * k + 1.0) / (2.0 * BL))
    fwd = np.concatenate([np.cos(ang), np.sin(ang)], axis=1)
    inv = np.concatenate([np.cos(ang).T, np.sin(ang).T], axis=0) / BL

    def pack(a):
        u = a.astype(np.float32).view(np.uint32).astype(np.uint64)
        h = ((u + 0x7FFF + ((u >> 16) & 1)) >> 16).astype(np.uint32)
        return h[0::2] | (h[1::2] << 16)

    return pack(fwd), pack(inv)


def _dot(a, b):
    return jnp.dot(a, b, preferred_element_type=F32)


def _dot_nt(a, b):
    return lax.dot_general(a, b, _NT_DIMS, preferred_element_type=F32)


def _pack(x):
    return pltpu.bitcast(x.astype(BF16), U32)


def _unpack(x):
    return pltpu.bitcast(x, BF16)


def _tree(ps):
    while len(ps) > 1:
        nxt = [ps[i] + ps[i + 1] for i in range(0, len(ps) - 1, 2)]
        if len(ps) % 2:
            nxt.append(ps[-1])
        ps = nxt
    return ps[0]


def _private(i, j):
    return i + lax.shift_right_logical(i + j, 16)


def _recip(x):
    r = pl.reciprocal(x, approx=True)
    return r * (2.0 - x * r)


def _features(p, mid, low, odd2):
    v = [p[8 * a:8 * (a + 1)] for a in range(4)] + [mid] + [p[8 * a:8 * (a + 1)] for a in range(4, 8)]

    def reduce(op, w):
        a = op(op(w[0], w[1]), op(w[2], w[3]))
        b = op(op(w[5], w[6]), op(w[7], w[8]))
        m = op(jnp.where(low, a, b), pltpu.roll(jnp.where(low, b, a), 4, 0))
        m = op(m, w[4])
        return op(m, jnp.where(odd2, pltpu.roll(m, 2, 0), pltpu.roll(m, 6, 0)))

    def spread(m):
        r = pltpu.roll(m, 4, 0)
        ma, mb = jnp.where(low, m, r), jnp.where(low, r, m)
        return [ma] * 4 + [m] + [mb] * 4

    mx = spread(reduce(jnp.maximum, v))
    mn = spread(reduce(jnp.minimum, v))
    ep = [jnp.exp2(a - m) for a, m in zip(v, mx)]
    en = [jnp.exp2(m - a) for a, m in zip(v, mn)]
    pp = [a * r for a, r in zip(ep, spread(_recip(reduce(jnp.add, ep))))]
    pn = [a * r for a, r in zip(en, spread(_recip(reduce(jnp.add, en))))]
    return jnp.concatenate(pp[0:4] + pn[0:4] + [pp[4], pn[4]] + pp[5:9] + pn[5:9], axis=0)


def _kernel(x_hbm, k_hbm, v_hbm, sk_hbm, h_hbm, d_hbm, wqkv_hbm, wp_hbm, wo_hbm, gate_hbm,
            f_hbm, g_hbm, out_hbm,
            xbuf, kbuf, vbuf, hbuf, wqkv, wo, skb, db, gb, wpb,
            wp2, a2b, wt, wot, wb, gwb, fmp, gmp, uh0, uh1, pr0, pr1, kvacc, k3,
            phi, vtb, lhs, gpb, obuf,
            sem_small, sem_w, sem_c, sem_o, bar):
    uhs = (uh0, uh1)
    praw = (pr0, pr1)
    small = [
        pltpu.make_async_copy(wp_hbm, wpb, sem_small),
        pltpu.make_async_copy(sk_hbm, skb, sem_small),
        pltpu.make_async_copy(d_hbm, db, sem_small),
        pltpu.make_async_copy(gate_hbm, gb, sem_small),
    ]

    def cp_kvh(c):
        rows = pl.ds(c * RC, RC)
        return [pltpu.make_async_copy(k_hbm.at[0, rows, :], kbuf.at[c], sem_c.at[c]),
                pltpu.make_async_copy(v_hbm.at[0, rows, :], vbuf.at[c], sem_c.at[c]),
                pltpu.make_async_copy(h_hbm.at[rows, :], hbuf.at[c], sem_c.at[c])]

    def cp_x(c, sem):
        return pltpu.make_async_copy(x_hbm.at[0, :, pl.ds(c * TS, TS)], xbuf.at[c, pl.ds(0, D), :], sem)

    def cp_step(c):
        return [cp_x(c, sem_c.at[c + 1])] + cp_kvh(c + 1)

    def cp_o(i, part):
        if part is None:
            rows = pl.ds(0, D)
        else:
            lo = PR * (OSPLIT[part - 1] if part else 0)
            rows = pl.ds(lo, PR * OSPLIT[part] - lo)
        return pltpu.make_async_copy(obuf.at[i, rows, :], out_hbm.at[0, rows, pl.ds(i * TS, TS)], sem_o)

    wcols = [(0, 384), (384, 256), (640, 2 * D - 640), (2 * D, D)]
    cp_w = [pltpu.make_async_copy(wqkv_hbm.at[:, pl.ds(a, n)], wqkv.at[:, pl.ds(a, n)], sem_w.at[j])
            for j, (a, n) in enumerate(wcols)]
    cp_b1 = [cp_x(0, sem_w.at[1]), cp_w[1]]
    cp_b3 = [pltpu.make_async_copy(f_hbm, fmp, sem_c.at[0])] + cp_kvh(0)
    cp_b5 = cp_kvh(1) + [cp_x(1, sem_c.at[1])]
    cp_late = [pltpu.make_async_copy(wo_hbm, wo, sem_w.at[4]), pltpu.make_async_copy(g_hbm, gmp, sem_w.at[4])]

    def fresh_region():
        def tick(_, c):
            pl.semaphore_signal(bar, 1)
            pl.semaphore_wait(bar, 1)
            return c
        lax.fori_loop(0, 2, tick, 0)

    batches = ([small, [cp_w[0]], cp_b1, [cp_w[2]], cp_b3, [cp_w[3]], cp_b5, cp_kvh(2)]
               + [cp_step(c) for c in range(2, NS)] + [cp_late])
    for batch in batches:
        for c in batch:
            c.start()
        pl.semaphore_signal(bar, 1)
        pl.semaphore_wait(bar, 1)
    for comp in range(3):
        k3[0, (3 * comp + 1) * D:(3 * comp + 2) * D, :] = jnp.zeros((D, BL), F32)
    for c in small:
        c.wait()

    lane8 = lax.broadcasted_iota(jnp.int32, (8, 128), 1)
    sub8 = lax.broadcasted_iota(jnp.int32, (8, 128), 0)
    low = sub8 < 4
    odd2 = (sub8 & 2) != 0

    def conv_au(c, uh):
        nj = JR // 8
        for p in range(RC // 8):
            lo = p * 8
            r1p = jnp.zeros((8, 128), F32)
            r2p = jnp.zeros((8, 128), F32)
            for a0 in range(0, NB, nj):
                w0, w1, w2, w3 = [wb[j, c, lo:lo + 8, :] for j in range(4)]
                us = []
                for i in range(a0, a0 + nj):
                    kt = kbuf[c, lo:lo + 8, i * BL:(i + 1) * BL].astype(F32)
                    vt = vbuf[c, lo:lo + 8, i * BL:(i + 1) * BL].astype(F32)
                    r1 = pltpu.roll(kt, 1, 1)
                    k1 = jnp.where(lane8 >= 1, r1, r1p)
                    t = w2 * kt + w3 * k1
                    r2 = pltpu.roll(t, 2, 1)
                    t2 = jnp.where(lane8 >= 2, r2, r2p)
                    ks = w0 * kt + w1 * k1 + t2
                    us.append(ks * vt)
                    r1p, r2p = r1, r2
                ur = _dot(jnp.concatenate(us, axis=0).astype(BF16), _unpack(fmp[...]))
                prev = None
                for i in range(a0, a0 + nj):
                    a = ur[8 * (i - a0):8 * (i - a0 + 1), 0:128]
                    b = ur[8 * (i - a0):8 * (i - a0 + 1), 128:256]
                    vals = (a + b, a, b)
                    for comp in range(3):
                        uh[p, comp, HB * (i % 2) + i // 2] = vals[comp]
                        if i % 2:
                            uh[p, comp, 2 * HB + i // 2] = vals[comp] + prev[comp]
                    prev = vals
                yield

    def conv_ah(c, uh):
        nj = JR // 16
        for rs in range(RC // 16):
            cp = dp = prev = None
            for a0 in range(0, NB, nj):
                hr = _dot(jnp.concatenate([hbuf[c, rs * 16:(rs + 1) * 16, i * BL:(i + 1) * BL]
                                           for i in range(a0, a0 + nj)], axis=0), _unpack(fmp[...]))
                for i in range(a0, a0 + nj):
                    cc = hr[16 * (i - a0):16 * (i - a0 + 1), 0:128]
                    dd = hr[16 * (i - a0):16 * (i - a0 + 1), 128:256]
                    if i == 0:
                        cc = cc + wb[4, c, rs * 16:(rs + 1) * 16, :]
                        c2, d2 = cc, dd
                    else:
                        c2, d2 = cc + dp, dd - cp
                    vals = (c2, d2 - c2, c2 + d2)
                    for comp in range(3):
                        outs = [(HB * (i % 2) + i // 2, vals[comp])]
                        if i % 2:
                            outs.append((2 * HB + i // 2, vals[comp] + prev[comp]))
                        for slot, val in outs:
                            uh[2 * rs, comp, 3 * HB + slot] = val[0:8]
                            uh[2 * rs + 1, comp, 3 * HB + slot] = val[8:16]
                    prev = vals
                    cp, dp = cc, dd
                yield

    def conv_b(crow, n, uh, m_lo=0, m_hi=HB):
        p, comp, r = n // 9, (n // 3) % 3, n % 3
        r0 = crow + ((3 * comp + r) * D + p * 8)
        if not isinstance(r0, int):
            r0 = pl.multiple_of(r0, 8)
        xs = [uh[p, comp, HB * r + i] for i in range(m_hi)]
        hs = [uh[p, comp, 3 * HB + HB * r + i] for i in range(m_hi)]
        for m in range(m_lo, m_hi):
            k3[m + 1, pl.ds(r0, 8), :] = _tree([xs[i] * hs[m - i] for i in range(m + 1)])

    eye = (lax.broadcasted_iota(jnp.int32, (32, 32), 0)
           == lax.broadcasted_iota(jnp.int32, (32, 32), 1)).astype(BF16)
    for e in range(DH):
        t = _dot_nt(eye, wpb[e])
        wp2[pl.ds(e, 32, stride=DH), :] = t
        wp2[pl.ds(D + e, 32, stride=DH), :] = t
    def row_map(r):
        shared = ((r >= 64) & (r < 72)) | (r >= OR)
        rr = jnp.where(r >= 72, r - 8, r)
        f = jnp.where(r >= OR, DH - 1, jnp.where(shared, 16, (rr & 31) >> 1))
        pair = jnp.where(shared, ((r >> 2) & 1) + (r & 2), rr >> 5)
        return f, 2 * pair + (r & 1)

    frow, _ = row_map(lax.broadcasted_iota(jnp.int32, (FR, DH), 0))
    rep = (lax.broadcasted_iota(jnp.int32, (FR, DH), 1) == frow).astype(BF16)
    a2b[...] = _dot_nt(rep, wp2[...].astype(BF16))
    _, hrow8 = row_map(lax.broadcasted_iota(jnp.int32, (FR, 128), 0))
    rel = lax.broadcasted_iota(jnp.int32, (FR, 128), 1) - hrow8 * DH
    subd = lax.broadcasted_iota(jnp.int32, (8, D), 0)
    parts = {}
    refs = {}
    wt_done = set()

    def unit_pair(a):
        return 4 if a in (8, OR // 8) else (a if a < 8 else a - 1) // 4

    def unit_cols(o, a):
        pair = unit_pair(a)
        if pair == 4:
            return 2 * GR * o, 2 * GR * (o + 1)
        return 2 * GR * o + 2 * DH * pair, 2 * GR * o + 2 * DH * (pair + 1)

    def fold(t):
        units = [(o, a) for o in range(8) for a in range(FR // 8)
                 if unit_cols(o, a)[0] < 128 * (t + 1) and unit_cols(o, a)[1] > 128 * t]
        units.sort(key=lambda u: (u[0], u[1] < OR // 8, u[1]))
        at = a2b[:, 128 * t:128 * (t + 1)]
        blocks = []
        for o, a in units:
            lo = 2 * GR * o - 128 * t
            rows = slice(8 * a, 8 * (a + 1))
            blocks.append(jnp.where((rel[rows] >= lo) & (rel[rows] < lo + DH), at[rows], 0.0))
        lt = jnp.concatenate(blocks, axis=0).astype(BF16)
        res = _dot_nt(lt, wqkv[:, 128 * t:128 * (t + 1)])
        for n, u in enumerate(units):
            piece = res[8 * n:8 * (n + 1)]
            parts[u] = piece if u not in parts else parts[u] + piece
        for o in range(8):
            if o not in refs and 2 * GR * (o + 1) <= 128 * (t + 1):
                r = parts.pop((o, OR // 8))
                ab = jnp.where((subd & 2) != 0, pltpu.roll(r, 2, 0), r)
                cd = jnp.where((subd & 2) != 0, r, pltpu.roll(r, 6, 0))
                ba, dc = pltpu.roll(ab, 4, 0), pltpu.roll(cd, 4, 0)
                refs[o] = [jnp.where(subd < 4, ab, ba), jnp.where(subd < 4, ba, ab),
                           jnp.where(subd < 4, cd, dc), jnp.where(subd < 4, dc, cd), r]
        for w in range(QK // 16):
            us = [divmod(u, OR // 8) for u in (2 * w, 2 * w + 1)]
            if w not in wt_done and all(o in refs for o, _ in us):
                both = jnp.concatenate([parts.pop((o, a)) - refs[o][unit_pair(a)] for o, a in us], axis=0)
                wt[8 * w:8 * (w + 1), :] = _pack(both * LOG2E)
                wt_done.add(w)

    cp_w[0].wait()
    for t in range(FQ):
        fold(t)

    def soft(slot, n, pr):
        g, q = n // NQ, n % NQ
        cols = slice(128 * q, 128 * (q + 1))
        r0 = OR * (g // 2)
        if g % 2 == 0:
            mid = jnp.where(odd2, 0.0, pr[r0 + 64:r0 + 72, cols])
            ph = _features(pr[r0:r0 + 64, cols], mid, low, odd2)
        else:
            mid = jnp.where(odd2, pr[QK + 8 * (g // 2):QK + 8 * (g // 2 + 1), cols], 0.0)
            ph = _features(pr[r0 + 72:r0 + OR, cols], mid, low, odd2)
        phi.at[slot][GR * g:GR * (g + 1), cols] = _pack(ph)

    def gpart(cs, n):
        rows = slice(GP * n, GP * (n + 1))
        gw = jnp.concatenate([gwb[rows, :]] * NQ, axis=1)
        for c in cs:
            xf = xbuf[c, rows, :].astype(F32)
            gpb[c, n] = jnp.sum((xf * gw).reshape(GP // 8, 8, TS), axis=0)

    def body1(i, par, name, cnt=None, ac=None):
        xt = xbuf[i, 0:D, :]
        if isinstance(i, int):
            crow, kslot = i * RC, i - 1
        else:
            crow = _private(i, 1) * RC
            kslot = _private(i, 2) - 1

        def proj(base, n):
            j, q = n // NQ, n % NQ
            base = base + j * (P1 // 2)
            r = _dot(_unpack(wt[base:base + P1 // 2, :]), xt[:, 128 * q:128 * (q + 1)])
            return r, j, slice(128 * q, 128 * (q + 1))

        ac = ac or (i + 1, uhs[1 - par])
        gen_u = conv_au(*ac)
        gen_h = conv_ah(*ac)
        cnt = cnt if cnt is not None else dict.fromkeys('vquhfBSG', 0)
        for tok in ORDER[name].split():
            kind = tok[0]
            n = cnt[kind]
            cnt[kind] += 1
            if kind == 'v':
                r, j, cols = proj(QK // 2, n)
                vtb.at[i][(P1 // 2) * j:(P1 // 2) * (j + 1), cols] = _pack(r)
            elif kind == 'q':
                assert all(w in wt_done for w in range((n // NQ) * (P1 // 16), (n // NQ + 1) * (P1 // 16)))
                r, j, cols = proj(0, n)
                praw[1 - par][P1 * j:P1 * (j + 1), cols] = r
                for o in range(8):
                    a = OR * o + 64 - P1 * j
                    if 0 <= a < P1:
                        praw[1 - par][QK + 8 * o:QK + 8 * (o + 1), cols] = r[a:a + 8]
            elif kind == 'u':
                next(gen_u)
            elif kind == 'h':
                next(gen_h)
            elif kind == 'f':
                fold(FQ + n)
            for ch in tok[1:]:
                n = cnt[ch]
                cnt[ch] += 1
                if ch == 'B':
                    conv_b(crow, 2 * n, uhs[par])
                    conv_b(crow, 2 * n + 1, uhs[par])
                elif ch == 'S':
                    soft(kslot, n, praw[par])
                elif ch == 'G':
                    gpart((0, 1), n)

    cnt0 = dict.fromkeys('vquhfBSG', 0)
    for c in cp_b1:
        c.wait()
    body1(0, 0, 's1', cnt0)
    cp_w[2].wait()
    body1(0, 0, 's2', cnt0)
    sk = skb[...].astype(F32)
    for j in range(4):
        wb[j] = jnp.broadcast_to(sk[j:j + 1, :], (128, D)).T.reshape(NC, RC, 128)
    wb[4] = jnp.broadcast_to(db[...].astype(F32).reshape(1, D), (128, D)).T.reshape(NC, RC, 128)
    gwb[...] = jnp.broadcast_to(gb[...].astype(F32).reshape(1, D), (128, D)).T
    for c in cp_b3:
        c.wait()
    body1(0, 0, 's3', cnt0, (0, uh0))
    cp_w[3].wait()
    fresh_region()
    body1(0, 0, 's4', cnt0)
    wt[QK // 2:(QK + D) // 2, :] = _pack(wqkv[:, 2 * D:3 * D].T)
    for c in cp_b5:
        c.wait()
    fresh_region()
    body1(0, 0, 's5', cnt0)
    for c in cp_kvh(2):
        c.wait()

    assert cnt0 == dict(v=18, q=34, u=32, h=32, f=NT - FQ, B=36, S=0, G=D // GP)

    def loop1(i, carry):
        for par in range(2):
            pl.when((i & 1) == par)(lambda par=par: body1(i, par, 'loop'))

        @pl.when(i + 1 < NS)
        def _():
            for c in cp_step(i + 1):
                c.wait()

        @pl.when(i + 1 == NS)
        def _():
            for c in cp_late:
                c.wait()

        return carry

    lax.fori_loop(1, NS, loop1, 0)

    def gfin(c):
        gl = _tree([gpb[c, n] for n in range(D // GP)])
        gl = gl + pltpu.roll(gl, 4, 0)
        gl = gl + pltpu.roll(gl, 2, 0)
        gl = gl + pltpu.roll(gl, 1, 0)
        return 1.0 / (1.0 + jnp.exp(-gl))

    def wo_t(c):
        n = min(128, D - 128 * c)
        wot[64 * c:64 * c + n // 2, :] = _pack(wo[:, 128 * c:128 * c + n].T)

    def b_last(m_lo, m_hi, per):
        return [lambda a=a: [conv_b((NC - 1) * RC, n, uh0, m_lo, m_hi) for n in range(a, min(a + per, 72))]
                for a in range(0, 72, per)]

    def weave(name, ms, queues):
        toks = ORDER[name].split() if queues else ['m'] * len(ms)
        assert len(toks) == len(ms)
        for fn, tok in zip(ms, toks):
            fn()
            for ch in tok[1:]:
                queues[int(ch)].pop(0)()
        assert not any(queues)

    def pair_rows(p):
        return GR * (p // 2) + 32 * (p % 2), (2 * DH * p // 16) * 16, (5 if p % 4 < 2 else 0)

    sub24 = lax.broadcasted_iota(jnp.int32, (KW // 2, TS), 0)
    accs = {}

    def kv_piece(p, c, first, last):
        fr, w0, sv = pair_rows(p)
        spare = (sub24 >= 4 * sv) & (sub24 < 4 * sv + 4)
        lv = jnp.concatenate(
            [_unpack(jnp.where(spare, jnp.uint32(0x3F803F80), vtb[c + a, w0 // 2:(w0 + KW) // 2, :]))
             for a in range(2)], axis=1)
        rv = jnp.concatenate([_unpack(phi[c + a, D + fr:D + fr + KF // 2, :]) for a in range(2)], axis=1)
        part = _dot_nt(lv, rv)
        if c == 0:
            acc = part
        elif first:
            acc = kvacc[KW * p:KW * (p + 1), :] + part
        else:
            acc = accs[p] + part
        accs[p] = acc
        if c == NS - 2:
            col = lax.broadcasted_iota(jnp.int32, (KW, KF), 1)
            row = lax.broadcasted_iota(jnp.int32, (KW, KF), 0)
            if p % 2 == 0:
                valid = (col < 64) | ((col & 7) < 4)
            else:
                valid = (col >= 16) | ((col & 7) >= 4)
            rr = row - (2 * DH * p - w0)
            hrow = jnp.where((rr >= 0) & (rr < 2 * DH), jnp.where(rr >= DH, 1, 0), -1)
            srow = row - 8 * sv
            hrow = jnp.where((srow >= 0) & (srow < 8), jnp.where(srow >= (2 if p % 2 == 0 else 6), 1, 0), hrow)
            lhs[(KW // 2) * p:(KW // 2) * (p + 1), :] = _pack(jnp.where(valid & (hrow == (col & 1)), acc, 0.0))
        elif last:
            kvacc[KW * p:KW * (p + 1), :] = acc

    def kv_pieces(c0, c1):
        return [lambda p=p, c=c: kv_piece(p, c, c == c0, c == c1 - 2)
                for p in range(NPAIR) for c in range(c0, c1, 2)]

    def chunk_pieces(i, lead):
        st = {'o': [], 'ts': {}}

        def num(g):
            for p in (2 * g, 2 * g + 1):
                fr, _, sv = pair_rows(p)
                res = _dot(_unpack(lhs[(KW // 2) * p:(KW // 2) * (p + 1), :]),
                           _unpack(phi[i, fr:fr + KF // 2, :]))
                rd = _recip(res[8 * sv:8 * (sv + 1)] + 1e-6)
                ra = jnp.broadcast_to(rd[0:1], (8, TS))
                rb = jnp.broadcast_to(rd[7:8], (8, TS))
                o0 = 8 if sv == 0 else 0
                o = [res[o0 + 8 * a:o0 + 8 * (a + 1)] * r for a, r in enumerate((ra, ra, rd, rb, rb))]
                if p % 2:
                    o[0] = o[0] + st['o'].pop()
                st['o'] += o
            if g == NG - 1:
                st['ot'] = jnp.concatenate(st['o'], axis=0).astype(BF16)
                st['gate'] = jnp.concatenate([gfin(i)] * (PR // 8), axis=0)

        def cpiece(j):
            def spec(slot, r):
                ks = [k3[slot, (3 * comp + r) * D + PR * j:(3 * comp + r) * D + PR * (j + 1), :]
                      for comp in range(3)]
                return jnp.concatenate([ks[0] - ks[2], ks[0] + ks[1]], axis=1)

            p0 = spec(i + 1, 0)
            zs = [p0 + spec(i, 1), spec(i + 1, 2) - p0 - spec(i + 1, 1)]
            y = _dot(jnp.concatenate(zs, axis=0).astype(BF16), _unpack(gmp[...]))
            y = jnp.concatenate([y[PR * q:PR * (q + 1)] for q in range(NQ)], axis=1)
            st['ts'][j] = xbuf[i, PR * j:PR * (j + 1), :].astype(F32) * y

        def out(j):
            bt = _dot(_unpack(wot[(PR // 2) * j:(PR // 2) * (j + 1), :]), st['ot'])
            obuf[i, PR * j:PR * (j + 1), :] = (bt + st['gate'] * (st['ts'].pop(j) - bt)).astype(BF16)
            if i == NS - 1 and j + 1 in OSPLIT:
                cp_o(i, OSPLIT.index(j + 1)).start()
            if XN <= i < NS - 1 and j + 1 == NP:
                cp_o(i, None).start()

        nums = [lambda g=g: num(g) for g in range(NG)]
        outs = [lambda j=j: cpiece(j) for j in range(lead)]
        for j in range(NP):
            outs.append(lambda j=j: out(j))
            if j + lead < NP:
                outs.append(lambda j=j: cpiece(j + lead))
        return nums, outs

    def g_pieces(c0, c1):
        return [lambda n=n, c=c: gpart((c, c + 1), n) for c in range(c0, c1, 2) for n in range(D // GP)]

    weave('ma', kv_pieces(0, KVA),
          [[lambda n=n: soft(NS - 1, n, pr0) for n in range(NG * NQ, 2 * NG * NQ)], b_last(0, BM, 8),
           [lambda c=c: wo_t(c) for c in range(5)], g_pieces(2, XN)])
    for name, c0, c1 in (('x', 0, XN), ('y', XN, NS)):
        fresh_region()
        pcs = [chunk_pieces(c, 4 if c == c0 else 1) for c in range(c0, c1)]
        ms = (kv_pieces(KVA, NS) if c0 == 0 else []) + pcs[0][0]
        for c in range(c0, c1):
            outs = pcs[c - c0][1]
            nxt = pcs[c - c0 + 1][0] if c + 1 < c1 else []
            k = len(outs) - 4 - len(nxt)
            ms += outs[:k] + [e for pair in zip(outs[k:k + len(nxt)], nxt) for e in pair] + outs[k + len(nxt):]
        queues = []
        if c0 == 0:
            queues = [[lambda n=n: soft(NS - 1, n, pr0) for n in range(NG * NQ)], b_last(BM, HB, 3),
                      g_pieces(XN, NS)]
        weave(name, ms, queues)
        if c0 == 0:
            for c in range(c0, c1):
                cp_o(c, None).start()
    for i in range(NS - 1):
        cp_o(i, None).wait()
    for k in range(len(OSPLIT)):
        cp_o(NS - 1, k).wait()


@jax.jit
def pallas_gated_mix__ssm_conv_h3__linear_kernel_hedgehog__prompt_kernel(A_q, A_k, A_v, A_shift_k, A_ssm_k, A_ssm_D, B_x, B_wqkv, B_w_phi, B_wo, gate_w):
    del B_x
    fwd, inv = _dft_consts()
    xT = jnp.transpose(A_q, (0, 2, 1))
    kT = jnp.transpose(A_k, (0, 2, 1))
    vT = jnp.transpose(A_v, (0, 2, 1))
    skT = jnp.transpose(A_shift_k, (1, 0))
    wp = jnp.transpose(B_w_phi, (1, 2, 0))
    hbm = pl.BlockSpec(memory_space=pltpu.HBM)
    scratch = [
        pltpu.VMEM((NS, DP, TS), BF16),
        pltpu.VMEM((NC, RC, S), BF16),
        pltpu.VMEM((NC, RC, S), BF16),
        pltpu.VMEM((NC, RC, S), BF16),
        pltpu.VMEM((D, 3 * D), BF16),
        pltpu.VMEM((D, D), BF16),
        pltpu.VMEM((4, D), BF16),
        pltpu.VMEM((D,), BF16),
        pltpu.VMEM((D,), BF16),
        pltpu.VMEM((DH, DH, 32), BF16),
        pltpu.VMEM((2 * D, DH), F32),
        pltpu.VMEM((FR, 2 * D), F32),
        pltpu.VMEM(((QK + D) // 2, D), U32),
        pltpu.VMEM((D // 2, D), U32),
        pltpu.VMEM((5, NC, RC, 128), F32),
        pltpu.VMEM((D, 128), F32),
        pltpu.VMEM((BL // 2, 2 * BL), U32),
        pltpu.VMEM((BL, BL), U32),
        pltpu.VMEM((RC // 8, 3, 6 * HB, 8, BL), F32),
        pltpu.VMEM((RC // 8, 3, 6 * HB, 8, BL), F32),
        pltpu.VMEM((QK + 64, TS), F32),
        pltpu.VMEM((QK + 64, TS), F32),
        pltpu.VMEM((NPAIR * KW, KF), F32),
        pltpu.VMEM((HB + 1, 9 * D, BL), F32),
        pltpu.VMEM((NS, 2 * DP, TS), U32),
        pltpu.VMEM((NS, DP // 2, TS), U32),
        pltpu.VMEM((NPAIR * KW // 2, KF), U32),
        pltpu.VMEM((NS, D // GP, 8, TS), F32),
        pltpu.VMEM((NS, D, TS), BF16),
        pltpu.SemaphoreType.DMA(()),
        pltpu.SemaphoreType.DMA((5,)),
        pltpu.SemaphoreType.DMA((NC,)),
        pltpu.SemaphoreType.DMA(()),
        pltpu.SemaphoreType.REGULAR(()),
    ]
    outT = pl.pallas_call(
        _kernel,
        out_shape=jax.ShapeDtypeStruct((1, D, S), BF16),
        in_specs=[hbm] * 12,
        out_specs=hbm,
        scratch_shapes=scratch,
        compiler_params=pltpu.CompilerParams(vmem_limit_bytes=100 * 1024 * 1024),
    )(xT, kT, vT, skT, A_ssm_k, A_ssm_D, B_wqkv, wp, B_wo, gate_w,
      jnp.asarray(fwd), jnp.asarray(inv))
    return jnp.transpose(outT, (0, 2, 1))
```
